```python
import jax
import jax.numpy as jnp

def _softmax(x, axis=-1):
    return jax.nn.softmax(x, axis=axis)
def _gelu(x):
    return jax.nn.gelu(x, approximate=True)
def _silu(x):
    return jax.nn.silu(x)
def _sigmoid(x):
    return jax.nn.sigmoid(x)
def _layernorm(x, axis=-1, eps=1e-5):
    m = jnp.mean(x, axis=axis, keepdims=True)
    v = jnp.var(x, axis=axis, keepdims=True)
    return (x - m) / jnp.sqrt(v + eps)
def _scatter_add(tgt, idx, src, axis=0):
    return tgt.at[idx].add(src)
def _segment_sum(src, seg, n):
    return jax.ops.segment_sum(src, seg, n)
class _Rng:
    def __init__(self, key):
        self._k = key
    def _next(self):
        self._k, sub = jax.random.split(self._k)
        return sub
    def normal(self, shape):
        return jax.random.normal(self._next(), shape, dtype=jnp.bfloat16)
    def randint(self, lo, hi, shape):
        return jax.random.randint(self._next(), shape, lo, hi, dtype=jnp.int32)
    def uniform(self, shape, lo=0.0, hi=1.0):
        return jax.random.uniform(self._next(), shape, jnp.bfloat16, lo, hi)
    def permutation(self, n):
        return jax.random.permutation(self._next(), n)


kernel_name = 'parallel_sum__gqa_block_cached__moe_arch_mod__decode'

def setup_inputs():
    _rng = _Rng(jax.random.key(int.from_bytes(__import__("os").urandom(4), "little")))
    _w = (lambda a: (lambda t: t.astype(jnp.bfloat16) if jnp.issubdtype(t.dtype, jnp.floating) else t)(jnp.asarray(a)))
    def _A_setup():
        B, Sq, D = 1, 1, 448
        Hq, Hkv, Sk, Dh = 16, 8, 65536, 256
        assert Hq % Hkv == 0, (Hq, Hkv)
        return {
            "x": _w((lambda *s: _rng.normal(s) * 0.05)(B, Sq, D)),
            "k_cache": _w((lambda *s: _rng.normal(s) * 0.05)(B, Hkv, Sk, Dh)),
            "v_cache": _w((lambda *s: _rng.normal(s) * 0.05)(B, Hkv, Sk, Dh)),
            "wq": _w((lambda *s: _rng.normal(s) * 0.05)(D, Hq * Dh) * (D ** -0.5)),
            "wo": _w((lambda *s: _rng.normal(s) * 0.05)(Hq * Dh, D) * ((Hq * Dh) ** -0.5)),
        }
    _A_in = _A_setup()

    def _B_setup():
        B, S, D, F, C = 1, 1, 448, 1792, 1
        return {
            "x": _w((lambda *s: _rng.normal(s) * 0.05)(B, S, D)),
            "w_r": _w((lambda *s: _rng.normal(s) * 0.05)(D)),
            "w_gate": _w((lambda *s: _rng.normal(s) * 0.05)(D, F)),
            "w_up": _w((lambda *s: _rng.normal(s) * 0.05)(D, F)),
            "w_down": _w((lambda *s: _rng.normal(s) * 0.05)(F, D)),
        }
    _B_in = _B_setup()

    return {
        "A_x": _A_in["x"],
        "A_k_cache": _A_in["k_cache"],
        "A_v_cache": _A_in["v_cache"],
        "A_wq": _A_in["wq"],
        "A_wo": _A_in["wo"],
        "B_x": _B_in["x"],
        "B_w_r": _B_in["w_r"],
        "B_w_gate": _B_in["w_gate"],
        "B_w_up": _B_in["w_up"],
        "B_w_down": _B_in["w_down"],
    }

def reference(A_x, A_k_cache, A_v_cache, A_wq, A_wo, B_x, B_w_r, B_w_gate, B_w_up, B_w_down):
    def _A_ref(x, k_cache, v_cache, wq, wo):
        B, Sq, D = x.shape
        Hq, Dh = 16, 256
        Hkv = k_cache.shape[1]
        rep = Hq // Hkv
        q = (lambda x, *d: x.transpose(*d))((x @ wq).reshape(B, Sq, Hq, Dh), 0, 2, 1, 3)
        k = jnp.repeat(k_cache, rep, axis=1)
        v = jnp.repeat(v_cache, rep, axis=1)
        scores = jnp.einsum("bhqd,bhkd->bhqk", q, k) * (Dh ** -0.5)
        p = _softmax(scores, axis=-1)
        o = jnp.einsum("bhqk,bhkd->bhqd", p, v)
        return (lambda x, *d: x.transpose(*d))(o, 0, 2, 1, 3).reshape(B, Sq, Hq * Dh) @ wo

    def _B_ref(x, w_r, w_gate, w_up, w_down):
        B, S, D = x.shape
        C = 1
        r = x @ w_r
        idx = jnp.argsort(-r, axis=-1)[:, :C]
        idx_e = jnp.repeat(idx.reshape(B, C, 1), D, axis=2)
        x_sel = jnp.take_along_axis(x, idx_e, axis=1)
        g = _silu(x_sel @ w_gate)
        u = x_sel @ w_up
        y = (g * u) @ w_down
        r_sel = _sigmoid(jnp.take_along_axis(r, idx, axis=1))
        y = y * r_sel.reshape(B, C, 1)
        b_off = (jnp.arange(B) * S).reshape(B, 1)
        flat_idx = (idx + b_off).reshape(B * C)
        zero = (x * 0.0).reshape(B * S, D)
        upd = _scatter_add(zero, flat_idx, y.reshape(B * C, D), axis=0)
        return x + upd.reshape(B, S, D)

    x = A_x
    xn = _layernorm(x, axis=-1)
    return x + _A_ref(xn, A_k_cache, A_v_cache, A_wq, A_wo) + _B_ref(xn, B_w_r, B_w_gate, B_w_up, B_w_down)
```

```python
import functools

import jax
import jax.numpy as jnp
from jax import lax
import jax.experimental.pallas as pl
import jax.experimental.pallas.tpu as pltpu

_HQ = 16
_DH = 256
_EPS = 1e-5
_NT = (((1,), (1,)), ((), ()))


def _make_kernel(*, hkv, sk, d, f, ch, ns, sub, nstr, piece):
    rep = _HQ // hkv
    nc = sk // ch
    total = hkv * nc
    ahead = ns - 1
    nsub = ch // sub
    npiece = ch // piece
    rows = 8
    f32 = jnp.float32
    bf16 = jnp.bfloat16

    def kernel(x_hbm, k_hbm, v_hbm, wq_hbm, wot_hbm, wr_hbm, wg_hbm, wu_hbm, wdt_hbm,
               o_hbm,
               x_v, wq_v, wo_v, wr_v, wg_v, wu_v, wd_v, q_s, out_v, kv,
               wsem, kvsem):
        def start_pairs(i, slot, js):
            base = (i // nc) * sk + lax.rem(i, nc) * (ch // nstr)
            base = pl.multiple_of(base, sub)
            for j in js:
                off = (j % nstr) * (sk // nstr) + (j // nstr) * sub
                for t, src in enumerate((k_hbm, v_hbm)):
                    pltpu.make_async_copy(
                        src.at[pl.ds(base + off, sub)],
                        kv.at[slot, t, pl.ds(j * sub, sub)],
                        kvsem.at[slot, t]).start(priority=t)

        def wait_chunk(slot, t):
            pltpu.make_async_copy(kv.at[slot, t], kv.at[slot, t], kvsem.at[slot, t]).wait()

        def halves(src, dst, sem):
            half = d // 2
            return [
                pltpu.make_async_copy(src.at[pl.ds(p * half, half)],
                                      dst.at[pl.ds(p * half, half)], sem.at[p])
                for p in range(2)
            ]

        cp_x = pltpu.make_async_copy(x_hbm, x_v, wsem.at[0, 0])
        cp_r = pltpu.make_async_copy(wr_hbm, wr_v, wsem.at[0, 1])
        cp_wq = halves(wq_hbm, wq_v, wsem.at[1])
        others = (halves(wg_hbm, wg_v, wsem.at[2]) + halves(wu_hbm, wu_v, wsem.at[3])
                  + halves(wdt_hbm, wd_v, wsem.at[4]))
        for h in range(hkv):
            others += halves(wot_hbm.at[:, pl.ds(h * rep * _DH, rep * _DH)], wo_v.at[h],
                             wsem.at[5 + h])
        cp_x.start(priority=0)
        cp_r.start(priority=1)
        for n, cp in enumerate(cp_wq):
            cp.start(priority=n % 2)
        for s in range(ahead):
            start_pairs(s, s, range(nsub))
        for n, cp in enumerate(others):
            cp.start(priority=n % 2)

        cp_x.wait()
        x = x_v[0].astype(f32)
        mean = jnp.mean(x, axis=-1, keepdims=True)
        xc = x - mean
        var = jnp.mean(xc * xc, axis=-1, keepdims=True)
        xn = (xc / jnp.sqrt(var + _EPS)).astype(bf16)
        xn8 = jnp.broadcast_to(xn, (rows, d))
        for cp in cp_wq:
            cp.wait()
        q_all = jnp.dot(xn8, wq_v[...], preferred_element_type=f32)
        q_all = q_all.astype(bf16).astype(f32) * (_DH ** -0.5)
        row = lax.broadcasted_iota(jnp.int32, (rows, _DH), 0)
        for h in range(hkv):
            qh = jnp.zeros((rows, _DH), f32)
            for r in range(rep):
                c0 = (h * rep + r) * _DH
                qh = jnp.where(row == r, q_all[:, c0:c0 + _DH], qh)
            q_s[h] = qh

        cp_r.wait()
        for cp in others:
            cp.wait()
        xnf = xn.astype(f32)
        wr = wr_v[...].astype(f32).reshape(1, d)
        r_logit = jnp.sum(xnf * wr, axis=-1, keepdims=True)
        g = jnp.dot(xn8, wg_v[...], preferred_element_type=f32)
        u = jnp.dot(xn8, wu_v[...], preferred_element_type=f32)
        hidden = (g * jax.nn.sigmoid(g) * u).astype(bf16)
        y = lax.dot_general(hidden, wd_v[...], _NT, preferred_element_type=f32)[0:1]
        base = x + (xnf + (xnf * 0.0 + y * jax.nn.sigmoid(r_logit)))

        def head_body(h, y_acc, last):
            q = q_s[h].astype(bf16)

            def chunk_body(c, carry, prefetch):
                m, l, acc = carry
                i = h * nc + c
                slot = lax.rem(i, ns)
                pslot = lax.rem(i + ahead, ns)
                todo = list(range(nsub)) if prefetch else []
                per_piece = -(-nsub // (2 * npiece))

                def issue():
                    js, todo[:] = todo[:per_piece], todo[per_piece:]
                    start_pairs(i + ahead, pslot, js)

                wait_chunk(slot, 0)
                ss = []
                for n in range(npiece):
                    kb = kv[slot, 0, pl.ds(n * piece, piece), :]
                    ss.append(lax.dot_general(q, kb, _NT, preferred_element_type=f32))
                    issue()
                m_new = m
                mx = functools.reduce(jnp.maximum, ss)
                m_new = jnp.maximum(m, jnp.max(mx, axis=-1, keepdims=True))
                alpha = jnp.exp(m - m_new)
                ps = [jnp.exp(s - m_new) for s in ss]
                l = alpha * l + jnp.sum(functools.reduce(jnp.add, ps), axis=-1, keepdims=True)
                acc = alpha * acc
                wait_chunk(slot, 1)
                for n in range(npiece):
                    vb = kv[slot, 1, pl.ds(n * piece, piece), :]
                    acc = acc + jnp.dot(ps[n].astype(bf16), vb, preferred_element_type=f32)
                    issue()
                assert not todo
                return m_new, l, acc

            carry = (jnp.full((rows, 1), -jnp.inf, f32), jnp.zeros((rows, 1), f32),
                     jnp.zeros((rows, _DH), f32))
            n_pre = nc - ahead if last else nc
            carry = lax.fori_loop(
                0, n_pre, functools.partial(chunk_body, prefetch=True), carry)
            if last:
                carry = lax.fori_loop(
                    n_pre, nc, functools.partial(chunk_body, prefetch=False), carry)
            _, l, acc = carry
            o = acc / l
            lhs = jnp.concatenate(
                [jnp.where(row == r, o, 0.0) for r in range(rep)], axis=1).astype(bf16)
            return y_acc + lax.dot_general(lhs, wo_v[h], _NT, preferred_element_type=f32)

        y_acc = lax.fori_loop(0, hkv - 1, functools.partial(head_body, last=False),
                              jnp.zeros((rows, d), f32))
        y_acc = head_body(hkv - 1, y_acc, last=True)
        attn = jnp.sum(y_acc, axis=0, keepdims=True)
        out_v[0] = (base + attn).astype(out_v.dtype)
        cp_o = pltpu.make_async_copy(out_v, o_hbm, wsem.at[0, 0])
        cp_o.start()
        cp_o.wait()

    return kernel


def _run(A_x, A_k_cache, A_v_cache, A_wq, A_wo, B_x, B_w_r, B_w_gate, B_w_up, B_w_down,
         *, ch=2048, ns=3, sub=64, nstr=32, piece=256, nobc=False):
    del B_x
    b, sq, d = A_x.shape
    _, hkv, sk, dh = A_k_cache.shape
    f = B_w_gate.shape[1]
    assert b == 1 and sq == 1 and dh == _DH and sk % ch == 0
    kernel = _make_kernel(hkv=hkv, sk=sk, d=d, f=f, ch=ch, ns=ns, sub=sub, nstr=nstr, piece=piece)
    hbm = pl.BlockSpec(memory_space=pltpu.HBM)
    pin = lambda a: pltpu.with_memory_space_constraint(a, pltpu.HBM)
    dt = A_x.dtype
    out = pl.pallas_call(
        kernel,
        out_shape=jax.ShapeDtypeStruct((b, sq, d), dt),
        in_specs=[hbm] * 9,
        out_specs=hbm,
        scratch_shapes=[
            pltpu.VMEM((b, sq, d), dt),
            pltpu.VMEM(A_wq.shape, dt),
            pltpu.VMEM((hkv, d, (_HQ // hkv) * dh), dt),
            pltpu.VMEM((d,), dt),
            pltpu.VMEM((d, f), dt),
            pltpu.VMEM((d, f), dt),
            pltpu.VMEM((d, f), dt),
            pltpu.VMEM((hkv, 8, dh), jnp.float32),
            pltpu.VMEM((b, sq, d), dt),
            pltpu.VMEM((ns, 2, ch, dh), dt),
            pltpu.SemaphoreType.DMA((5 + hkv, 2)),
            pltpu.SemaphoreType.DMA((ns, 2)),
        ],
        compiler_params=pltpu.CompilerParams(
            vmem_limit_bytes=100 * 1024 * 1024, disable_bounds_checks=nobc),
    )(
        pin(A_x),
        pin(A_k_cache.reshape(hkv * sk, dh)),
        pin(A_v_cache.reshape(hkv * sk, dh)),
        pin(A_wq), pin(A_wo.T),
        pin(B_w_r),
        pin(B_w_gate), pin(B_w_up), pin(B_w_down.T),
    )
    return out


@jax.jit
def pallas_parallel_sum__gqa_block_cached__moe_arch_mod__decode_kernel(
    A_x: jax.Array,
    A_k_cache: jax.Array,
    A_v_cache: jax.Array,
    A_wq: jax.Array,
    A_wo: jax.Array,
    B_x: jax.Array,
    B_w_r: jax.Array,
    B_w_gate: jax.Array,
    B_w_up: jax.Array,
    B_w_down: jax.Array,
):
    return _run(A_x, A_k_cache, A_v_cache, A_wq, A_wo, B_x, B_w_r, B_w_gate, B_w_up, B_w_down)
```

```python
import functools

import jax
import jax.numpy as jnp
from jax import lax
import jax.experimental.pallas as pl
import jax.experimental.pallas.tpu as pltpu

_HQ = 16
_DH = 256
_EPS = 1e-5
_NT = (((1,), (1,)), ((), ()))


def _make_kernel(*, hkv, sk, d, ns, sub, sph, shift, lag):
    rep = _HQ // hkv
    nstr = hkv * sph
    span = sk // sph
    total = span // sub
    ahead = ns - (2 if any(shift) else 1)
    f32 = jnp.float32
    bf16 = jnp.bfloat16

    def kernel(x_hbm, k_hbm, v_hbm, wq_hbm, wot_hbm, wr_hbm, wg_hbm, wu_hbm, wdt_hbm,
               o_hbm,
               x_v, wq_v, wo_v, wr_v, wg_v, wu_v, wd_v, q_s, out_v, kv,
               wsem, kvsem):
        kv_hbm = (k_hbm, v_hbm)

        def start_pairs(i, slot, js, final=False):
            base = pl.multiple_of(i * sub, sub)
            for j in js:
                for t in range(2):
                    n = sub - shift[t] if final else sub
                    pltpu.make_async_copy(
                        kv_hbm[t].at[pl.ds(base + (j * span + shift[t]), n)],
                        kv.at[slot, t, pl.ds(j * sub, n)],
                        kvsem.at[slot, t]).start(priority=t)

        def wait_rows(t, n, sem):
            buf = kv.at[0, t, pl.ds(0, n)]
            pltpu.make_async_copy(buf, buf, sem).wait()

        def load_keys(t, h, slot, prev):
            if not shift[t]:
                return kv[slot, t, pl.ds(h * sph * sub, sph * sub), :]
            parts = []
            for j in range(h * sph, (h + 1) * sph):
                parts.append(kv[prev, t, pl.ds((j + 1) * sub - shift[t], shift[t]), :])
                parts.append(kv[slot, t, pl.ds(j * sub, sub - shift[t]), :])
            return jnp.concatenate(parts, axis=0)

        def halves(src, dst, sem):
            half = d // 2
            return [
                pltpu.make_async_copy(src.at[pl.ds(p * half, half)],
                                      dst.at[pl.ds(p * half, half)], sem.at[p])
                for p in range(2)
            ]

        cp_x = pltpu.make_async_copy(x_hbm, x_v, wsem.at[0, 0])
        cp_r = pltpu.make_async_copy(wr_hbm, wr_v, wsem.at[0, 1])
        cp_wq = halves(wq_hbm, wq_v, wsem.at[1])
        others = (halves(wg_hbm, wg_v, wsem.at[2]) + halves(wu_hbm, wu_v, wsem.at[3])
                  + halves(wdt_hbm, wd_v, wsem.at[4]) + halves(wot_hbm, wo_v, wsem.at[5]))
        cp_x.start(priority=0)
        cp_r.start(priority=1)
        for n, cp in enumerate(cp_wq):
            cp.start(priority=n % 2)
        for t in range(2):
            for j in range(nstr if shift[t] else 0):
                pltpu.make_async_copy(
                    kv_hbm[t].at[pl.ds(j * span, shift[t])],
                    kv.at[ns - 1, t, pl.ds((j + 1) * sub - shift[t], shift[t])],
                    wsem.at[6, t]).start(priority=t)
        for s in range(ahead):
            start_pairs(s, s, range(nstr))

        cp_x.wait()
        x = x_v[0].astype(f32)
        mean = jnp.mean(x, axis=-1, keepdims=True)
        xc = x - mean
        var = jnp.mean(xc * xc, axis=-1, keepdims=True)
        xn = (xc / jnp.sqrt(var + _EPS)).astype(bf16)
        xn_b = jnp.broadcast_to(xn, (_HQ, d))
        for cp in cp_wq:
            cp.wait()
        q_all = jnp.dot(xn_b, wq_v[...], preferred_element_type=f32)
        q_all = q_all.astype(bf16).astype(f32) * (_DH ** -0.5)
        row = lax.broadcasted_iota(jnp.int32, (_HQ, _DH), 0)
        for h in range(hkv):
            qh = jnp.zeros((_HQ, _DH), f32)
            for r in range(h * rep, (h + 1) * rep):
                qh = jnp.where(row == r, q_all[:, r * _DH:(r + 1) * _DH], qh)
            q_s[h] = qh.astype(bf16)
        for t in range(2):
            if shift[t]:
                wait_rows(t, nstr * shift[t], wsem.at[6, t])

        kv_head = lax.broadcasted_iota(jnp.int32, (_HQ, sph * sub), 0) // rep

        def step(i, carry, prefetch, final=False):
            m, l, acc = carry
            slot = lax.rem(i, ns)
            prev = lax.rem(i + (ns - 1), ns)
            pslot = lax.rem(i + ahead, ns)
            todo = list(range(nstr)) if prefetch else []
            per_piece = -(-nstr // (2 * hkv))

            def issue():
                js, todo[:] = todo[:per_piece], todo[per_piece:]
                start_pairs(i + ahead, pslot, js, final=prefetch == "final")

            def wait(t):
                wait_rows(t, nstr * (sub - shift[t] if final else sub), kvsem.at[slot, t])

            wait(0)
            s = None
            for h in range(hkv):
                sh = lax.dot_general(q_s[h], load_keys(0, h, slot, prev), _NT,
                                     preferred_element_type=f32)
                s = sh if s is None else s + sh
                issue()
            m_new = jnp.maximum(m, jnp.max(s, axis=-1, keepdims=True))
            alpha = jnp.exp(m - m_new)
            p = jnp.exp(s - m_new)
            l = alpha * l + jnp.sum(p, axis=-1, keepdims=True)
            acc = alpha * acc
            wait(1)
            for h in range(hkv):
                ph = jnp.where(kv_head == h, p, 0.0).astype(bf16)
                acc = acc + jnp.dot(ph, load_keys(1, h, slot, prev),
                                    preferred_element_type=f32)
                issue()
            assert not todo
            return m_new, l, acc

        carry = (jnp.full((_HQ, 1), -jnp.inf, f32), jnp.zeros((_HQ, 1), f32),
                 jnp.zeros((_HQ, _DH), f32))

        def early(i, carry):
            for n in range(0, len(others), 2):
                @pl.when(i == (n // 2))
                def _():
                    others[n].start(priority=0)
                    others[n + 1].start(priority=1)
            return step(i, carry, True)

        n_pre = total - ahead
        carry = lax.fori_loop(0, lag, early, carry)

        cp_r.wait()
        for cp in others:
            cp.wait()
        xnf = xn.astype(f32)
        wr = wr_v[...].astype(f32).reshape(1, d)
        r_logit = jnp.sum(xnf * wr, axis=-1, keepdims=True)
        g = jnp.dot(xn_b, wg_v[...], preferred_element_type=f32)
        u = jnp.dot(xn_b, wu_v[...], preferred_element_type=f32)
        hidden = (g * jax.nn.sigmoid(g) * u).astype(bf16)
        y = lax.dot_general(hidden, wd_v[...], _NT, preferred_element_type=f32)[0:1]
        resid = x + (xnf + (xnf * 0.0 + y * jax.nn.sigmoid(r_logit)))

        carry = lax.fori_loop(lag, n_pre - 1, lambda i, c: step(i, c, True), carry)
        carry = step(n_pre - 1, carry, "final")
        carry = lax.fori_loop(n_pre, total - 1, lambda i, c: step(i, c, False), carry)
        _, l, acc = step(total - 1, carry, False, final=True)

        o = acc / l
        lhs = jnp.concatenate(
            [jnp.where(row == r, o, 0.0).astype(bf16) for r in range(_HQ)], axis=1)
        attn = lax.dot_general(lhs, wo_v[...], _NT, preferred_element_type=f32)
        out_v[0] = (resid + jnp.sum(attn, axis=0, keepdims=True)).astype(out_v.dtype)
        cp_o = pltpu.make_async_copy(out_v, o_hbm, wsem.at[0, 0])
        cp_o.start()
        cp_o.wait()

    return kernel


def _run(A_x, A_k_cache, A_v_cache, A_wq, A_wo, B_x, B_w_r, B_w_gate, B_w_up, B_w_down,
         *, ns=6, sub=64, sph=2, shift=(0, 32), lag=8):
    del B_x
    b, sq, d = A_x.shape
    _, hkv, sk, dh = A_k_cache.shape
    f = B_w_gate.shape[1]
    assert b == 1 and sq == 1 and dh == _DH and sk % (sph * sub) == 0
    kernel = _make_kernel(hkv=hkv, sk=sk, d=d, ns=ns, sub=sub, sph=sph, shift=shift, lag=lag)
    hbm = pl.BlockSpec(memory_space=pltpu.HBM)
    pin = lambda a: pltpu.with_memory_space_constraint(a, pltpu.HBM)
    dt = A_x.dtype
    out = pl.pallas_call(
        kernel,
        out_shape=jax.ShapeDtypeStruct((b, sq, d), dt),
        in_specs=[hbm] * 9,
        out_specs=hbm,
        scratch_shapes=[
            pltpu.VMEM((b, sq, d), dt),
            pltpu.VMEM(A_wq.shape, dt),
            pltpu.VMEM((d, _HQ * dh), dt),
            pltpu.VMEM((d,), dt),
            pltpu.VMEM((d, f), dt),
            pltpu.VMEM((d, f), dt),
            pltpu.VMEM((d, f), dt),
            pltpu.VMEM((hkv, _HQ, dh), dt),
            pltpu.VMEM((b, sq, d), dt),
            pltpu.VMEM((ns, 2, hkv * sph * sub, dh), dt),
            pltpu.SemaphoreType.DMA((7, 2)),
            pltpu.SemaphoreType.DMA((ns, 2)),
        ],
        compiler_params=pltpu.CompilerParams(vmem_limit_bytes=100 * 1024 * 1024),
    )(
        pin(A_x),
        pin(A_k_cache.reshape(hkv * sk, dh)),
        pin(A_v_cache.reshape(hkv * sk, dh)),
        pin(A_wq), pin(A_wo.T),
        pin(B_w_r),
        pin(B_w_gate), pin(B_w_up), pin(B_w_down.T),
    )
    return out


@jax.jit
def pallas_parallel_sum__gqa_block_cached__moe_arch_mod__decode_kernel(
    A_x: jax.Array,
    A_k_cache: jax.Array,
    A_v_cache: jax.Array,
    A_wq: jax.Array,
    A_wo: jax.Array,
    B_x: jax.Array,
    B_w_r: jax.Array,
    B_w_gate: jax.Array,
    B_w_up: jax.Array,
    B_w_down: jax.Array,
):
    return _run(A_x, A_k_cache, A_v_cache, A_wq, A_wo, B_x, B_w_r, B_w_gate, B_w_up, B_w_down)
```

```python
import functools

import jax
import jax.numpy as jnp
from jax import lax
import jax.experimental.pallas as pl
import jax.experimental.pallas.tpu as pltpu

_HQ = 16
_DH = 256
_EPS = 1e-5
_NT = (((1,), (1,)), ((), ()))


def _make_kernel(*, hkv, sk, d, ns, sub, sph, shift, lag):
    rep = _HQ // hkv
    nstr = hkv * sph
    span = sk // sph
    total = span // sub
    ahead = ns - (2 if any(shift) else 1)
    f32 = jnp.float32
    bf16 = jnp.bfloat16

    def kernel(x_hbm, k_hbm, v_hbm, wq_hbm, wot_hbm, wr_hbm, wg_hbm, wu_hbm, wdt_hbm,
               o_hbm,
               x_v, wq_v, wo_v, wr_v, wg_v, wu_v, wd_v, q_s, out_v, kv,
               wsem, kvsem):
        kv_hbm = (k_hbm, v_hbm)

        def start_pairs(i, slot, js, final=False):
            base = pl.multiple_of(i * sub, sub)
            for j in js:
                for t in range(2):
                    n = sub - shift[t] if final else sub
                    pltpu.make_async_copy(
                        kv_hbm[t].at[pl.ds(base + (j * span + shift[t]), n)],
                        kv.at[slot, t, pl.ds(j * sub, n)],
                        kvsem.at[slot, t]).start(priority=t)

        def wait_rows(slot, t, n, sem):
            buf = kv.at[slot, t, pl.ds(0, n)]
            pltpu.make_async_copy(buf, buf, sem).wait()

        def load_keys(t, h, slot, prev):
            if not shift[t]:
                return kv[slot, t, pl.ds(h * sph * sub, sph * sub), :]
            parts = []
            for j in range(h * sph, (h + 1) * sph):
                parts.append(kv[prev, t, pl.ds((j + 1) * sub - shift[t], shift[t]), :])
                parts.append(kv[slot, t, pl.ds(j * sub, sub - shift[t]), :])
            return jnp.concatenate(parts, axis=0)

        def halves(src, dst, sem):
            half = d // 2
            return [
                pltpu.make_async_copy(src.at[pl.ds(p * half, half)],
                                      dst.at[pl.ds(p * half, half)], sem.at[p])
                for p in range(2)
            ]

        cp_x = pltpu.make_async_copy(x_hbm, x_v, wsem.at[0, 0])
        cp_r = pltpu.make_async_copy(wr_hbm, wr_v, wsem.at[0, 1])
        cp_wq = halves(wq_hbm, wq_v, wsem.at[1])
        others = (halves(wg_hbm, wg_v, wsem.at[2]) + halves(wu_hbm, wu_v, wsem.at[3])
                  + halves(wdt_hbm, wd_v, wsem.at[4]) + halves(wot_hbm, wo_v, wsem.at[5]))
        cp_x.start(priority=0)
        cp_r.start(priority=1)
        for n, cp in enumerate(cp_wq):
            cp.start(priority=n % 2)
        for t in range(2):
            for j in range(nstr if shift[t] else 0):
                pltpu.make_async_copy(
                    kv_hbm[t].at[pl.ds(j * span, shift[t])],
                    kv.at[ns - 1, t, pl.ds((j + 1) * sub - shift[t], shift[t])],
                    wsem.at[6, t]).start(priority=t)
        for s in range(ahead):
            start_pairs(s, s, range(nstr))

        cp_x.wait()
        x = x_v[0].astype(f32)
        mean = jnp.mean(x, axis=-1, keepdims=True)
        xc = x - mean
        var = jnp.mean(xc * xc, axis=-1, keepdims=True)
        xn = (xc / jnp.sqrt(var + _EPS)).astype(bf16)
        xn_b = jnp.broadcast_to(xn, (_HQ, d))
        for cp in cp_wq:
            cp.wait()
        q_all = jnp.dot(xn_b, wq_v[...], preferred_element_type=f32)
        q_all = q_all.astype(bf16).astype(f32) * (_DH ** -0.5)
        row = lax.broadcasted_iota(jnp.int32, (_HQ, _DH), 0)
        for h in range(hkv):
            qh = jnp.zeros((_HQ, _DH), f32)
            for r in range(h * rep, (h + 1) * rep):
                qh = jnp.where(row == r, q_all[:, r * _DH:(r + 1) * _DH], qh)
            q_s[h] = qh.astype(bf16)
        for t in range(2):
            if shift[t]:
                wait_rows(ns - 1, t, nstr * shift[t], wsem.at[6, t])

        kv_head = lax.broadcasted_iota(jnp.int32, (_HQ, sph * sub), 0) // rep

        def step(i, carry, prefetch, final=False):
            m, l, acc = carry
            slot = lax.rem(i, ns)
            prev = lax.rem(i + (ns - 1), ns)
            pslot = lax.rem(i + ahead, ns)
            todo = list(range(nstr)) if prefetch else []
            per_piece = -(-nstr // (2 * hkv))

            def issue():
                js, todo[:] = todo[:per_piece], todo[per_piece:]
                start_pairs(i + ahead, pslot, js, final=prefetch == "final")

            def wait(t):
                wait_rows(slot, t, nstr * (sub - shift[t] if final else sub),
                          kvsem.at[slot, t])

            wait(0)
            s = None
            for h in range(hkv):
                sh = lax.dot_general(q_s[h], load_keys(0, h, slot, prev), _NT,
                                     preferred_element_type=f32)
                s = sh if s is None else s + sh
                issue()
            m_new = jnp.maximum(m, jnp.max(s, axis=-1, keepdims=True))
            alpha = jnp.exp(m - m_new)
            p = jnp.exp(s - m_new)
            l = alpha * l + jnp.sum(p, axis=-1, keepdims=True)
            acc = alpha * acc
            wait(1)
            for h in range(hkv):
                ph = jnp.where(kv_head == h, p, 0.0).astype(bf16)
                acc = acc + jnp.dot(ph, load_keys(1, h, slot, prev),
                                    preferred_element_type=f32)
                issue()
            assert not todo
            return m_new, l, acc

        carry = (jnp.full((_HQ, 1), -jnp.inf, f32), jnp.zeros((_HQ, 1), f32),
                 jnp.zeros((_HQ, _DH), f32))

        def early(i, carry):
            for n in range(0, len(others), 2):
                @pl.when(i == (n // 2))
                def _():
                    others[n].start(priority=0)
                    others[n + 1].start(priority=1)
            return step(i, carry, True)

        n_pre = total - ahead
        carry = lax.fori_loop(0, lag, early, carry)

        cp_r.wait()
        for cp in others:
            cp.wait()
        xnf = xn.astype(f32)
        wr = wr_v[...].astype(f32).reshape(1, d)
        r_logit = jnp.sum(xnf * wr, axis=-1, keepdims=True)
        g = jnp.dot(xn_b, wg_v[...], preferred_element_type=f32)
        u = jnp.dot(xn_b, wu_v[...], preferred_element_type=f32)
        hidden = (g * jax.nn.sigmoid(g) * u).astype(bf16)
        y = lax.dot_general(hidden, wd_v[...], _NT, preferred_element_type=f32)[0:1]
        resid = x + (xnf + (xnf * 0.0 + y * jax.nn.sigmoid(r_logit)))

        carry = lax.fori_loop(lag, n_pre - 1, lambda i, c: step(i, c, True), carry)
        carry = step(n_pre - 1, carry, "final")
        carry = lax.fori_loop(n_pre, total - 1, lambda i, c: step(i, c, False), carry)
        _, l, acc = step(total - 1, carry, False, final=True)

        o = acc / l
        lhs = jnp.concatenate(
            [jnp.where(row == r, o, 0.0).astype(bf16) for r in range(_HQ)], axis=1)
        attn = lax.dot_general(lhs, wo_v[...], _NT, preferred_element_type=f32)
        out_v[0] = (resid + jnp.sum(attn, axis=0, keepdims=True)).astype(out_v.dtype)
        cp_o = pltpu.make_async_copy(out_v, o_hbm, wsem.at[0, 0])
        cp_o.start()
        cp_o.wait()

    return kernel


def _run(A_x, A_k_cache, A_v_cache, A_wq, A_wo, B_x, B_w_r, B_w_gate, B_w_up, B_w_down,
         *, ns=6, sub=64, sph=2, shift=(0, 32), lag=8):
    del B_x
    b, sq, d = A_x.shape
    _, hkv, sk, dh = A_k_cache.shape
    f = B_w_gate.shape[1]
    assert b == 1 and sq == 1 and dh == _DH and sk % (sph * sub) == 0
    kernel = _make_kernel(hkv=hkv, sk=sk, d=d, ns=ns, sub=sub, sph=sph, shift=shift, lag=lag)
    hbm = pl.BlockSpec(memory_space=pltpu.HBM)
    pin = lambda a: pltpu.with_memory_space_constraint(a, pltpu.HBM)
    dt = A_x.dtype
    out = pl.pallas_call(
        kernel,
        out_shape=jax.ShapeDtypeStruct((b, sq, d), dt),
        in_specs=[hbm] * 9,
        out_specs=hbm,
        scratch_shapes=[
            pltpu.VMEM((b, sq, d), dt),
            pltpu.VMEM(A_wq.shape, dt),
            pltpu.VMEM((d, _HQ * dh), dt),
            pltpu.VMEM((d,), dt),
            pltpu.VMEM((d, f), dt),
            pltpu.VMEM((d, f), dt),
            pltpu.VMEM((d, f), dt),
            pltpu.VMEM((hkv, _HQ, dh), dt),
            pltpu.VMEM((b, sq, d), dt),
            pltpu.VMEM((ns, 2, hkv * sph * sub, dh), dt),
            pltpu.SemaphoreType.DMA((7, 2)),
            pltpu.SemaphoreType.DMA((ns, 2)),
        ],
        compiler_params=pltpu.CompilerParams(vmem_limit_bytes=100 * 1024 * 1024),
    )(
        pin(A_x),
        pin(A_k_cache.reshape(hkv * sk, dh)),
        pin(A_v_cache.reshape(hkv * sk, dh)),
        pin(A_wq), pin(A_wo.T),
        pin(B_w_r),
        pin(B_w_gate), pin(B_w_up), pin(B_w_down.T),
    )
    return out


@jax.jit
def pallas_parallel_sum__gqa_block_cached__moe_arch_mod__decode_kernel(
    A_x: jax.Array,
    A_k_cache: jax.Array,
    A_v_cache: jax.Array,
    A_wq: jax.Array,
    A_wo: jax.Array,
    B_x: jax.Array,
    B_w_r: jax.Array,
    B_w_gate: jax.Array,
    B_w_up: jax.Array,
    B_w_down: jax.Array,
):
    return _run(A_x, A_k_cache, A_v_cache, A_wq, A_wo, B_x, B_w_r, B_w_gate, B_w_up, B_w_down)
```
